```python
import os as _os
_os.environ.setdefault("JAX_PLATFORMS", "cpu")
import jax
import jax.numpy as jnp

def _softmax(x, axis=-1):
    return jax.nn.softmax(x, axis=axis)
def _gelu(x):
    return jax.nn.gelu(x, approximate=True)
def _silu(x):
    return jax.nn.silu(x)
def _sigmoid(x):
    return jax.nn.sigmoid(x)
def _layernorm(x, axis=-1, eps=1e-5):
    m = jnp.mean(x, axis=axis, keepdims=True)
    v = jnp.var(x, axis=axis, keepdims=True)
    return (x - m) / jnp.sqrt(v + eps)
def _scatter_add(tgt, idx, src, axis=0):
    return tgt.at[idx].add(src)
def _segment_sum(src, seg, n):
    return jax.ops.segment_sum(src, seg, n)
class _Rng:
    def __init__(self, key):
        self._k = key
    def _next(self):
        self._k, sub = jax.random.split(self._k)
        return sub
    def normal(self, shape):
        return jax.random.normal(self._next(), shape, dtype=jnp.bfloat16)
    def randint(self, lo, hi, shape):
        return jax.random.randint(self._next(), shape, lo, hi, dtype=jnp.int32)
    def uniform(self, shape, lo=0.0, hi=1.0):
        return jax.random.uniform(self._next(), shape, jnp.bfloat16, lo, hi)
    def permutation(self, n):
        return jax.random.permutation(self._next(), n)


kernel_name = 'concat_heads__softmax_full_mha__grouped_kv_mqa__prompt'

def setup_inputs():
    _rng = _Rng(jax.random.key(int.from_bytes(__import__("os").urandom(4), "little")))
    _w = (lambda a: (lambda t: t.astype(jnp.bfloat16) if jnp.issubdtype(t.dtype, jnp.floating) else t)(jnp.asarray(a)))
    def _A_setup():
        B, S, D = 1, 2048, 640
        return {
            "x": _w((lambda *s: _rng.normal(s) * 0.1)(B, S, D)),
            "wqkv": _w((lambda *s: _rng.normal(s) * 0.1)(D, 3 * D)),
            "wo": _w((lambda *s: _rng.normal(s) * 0.05)(D, D)),
        }
    _A_in = _A_setup()

    def _B_setup():
        B, S, D, H = 1, 2048, 640, 32
        Dh = D // H
        return {
            "x": _w((lambda *s: _rng.normal(s) * 0.05)(B, S, D)),
            "wq": _w((lambda *s: _rng.normal(s) * 0.4)(D, H * Dh)),
            "wk": _w((lambda *s: _rng.normal(s) * 0.4)(D, Dh)),
            "wv": _w((lambda *s: _rng.normal(s) * 0.05)(D, Dh)),
            "wo": _w((lambda *s: _rng.normal(s) * 0.05)(H * Dh, D)),
        }
    _B_in = _B_setup()

    return {
        "A_x": _A_in["x"],
        "A_wqkv": _A_in["wqkv"],
        "A_wo": _A_in["wo"],
        "B_x": _B_in["x"],
        "B_wq": _B_in["wq"],
        "B_wk": _B_in["wk"],
        "B_wv": _B_in["wv"],
        "B_wo": _B_in["wo"],
    }

def reference(A_x, A_wqkv, A_wo, B_x, B_wq, B_wk, B_wv, B_wo):
    def _A_ref(x, wqkv, wo):
        B, S, D = x.shape
        H = 32; Dh = D // H
        qkv = (lambda x, *d: x.transpose(*d))((x @ wqkv).reshape(B, S, 3, H, Dh), 2, 0, 3, 1, 4)
        q, k, v = qkv[0], qkv[1], qkv[2]
        scale = Dh ** -0.5
        scores = jnp.einsum("bhqd,bhkd->bhqk", q, k) * scale
        p = _softmax(scores, axis=-1)
        o = jnp.einsum("bhqk,bhkd->bhqd", p, v)
        return (lambda x, *d: x.transpose(*d))(o, 0, 2, 1, 3).reshape(B, S, D) @ wo

    def _B_ref(x, wq, wk, wv, wo):
        B, S, D = x.shape
        H = 32
        Dh = D // H
        q = (lambda x, *d: x.transpose(*d))((x @ wq).reshape(B, S, H, Dh), 0, 2, 1, 3)
        k = x @ wk
        v = x @ wv
        scores = jnp.einsum("bhqd,bkd->bhqk", q, k) * (Dh ** -0.5)
        p = _softmax(scores, axis=-1)
        o = jnp.einsum("bhqk,bkd->bhqd", p, v)
        return (lambda x, *d: x.transpose(*d))(o, 0, 2, 1, 3).reshape(B, S, H * Dh) @ wo

    a = _A_ref(A_x, A_wqkv, A_wo)
    b = _B_ref(B_x, B_wq, B_wk, B_wv, B_wo)
    return jnp.concatenate([a, b], axis=-1)
```

```python
import functools
import math

import jax
import jax.numpy as jnp
from jax import lax
import jax.experimental.pallas as pl
import jax.experimental.pallas.tpu as pltpu

S = 2048
D = 640
H = 32
DH = 20
GH = 6
NG = 6
GW = GH * DH
RP = 24
TQ = 512
TK = 256
QSCALE = (DH ** -0.5) * math.log2(math.e)
SAFE_BOUND = 48.0
F32 = jnp.float32
BF16 = jnp.bfloat16


def _bf(x):
    return x.astype(BF16).astype(F32)


def _kernel(xa_ref, wqkv_ref, woa_ref, xb_ref, wqb_ref, wkb_ref, wvb_ref, wob_ref,
            o_ref,
            qa_ref, ka_ref, vta_ref, qb_ref, kb_ref, vtb_ref,
            ota_ref, otb_ref, wopa_ref, wopb_ref, kmax_ref, flag_ref):
    step = pl.program_id(0)

    @pl.when(step == 0)
    def _prologue():
        lane = lax.broadcasted_iota(jnp.int32, (1, 128), 1)
        row24 = lax.broadcasted_iota(jnp.int32, (RP, 1), 0)
        ir = lax.broadcasted_iota(jnp.int32, (128, 128), 0)
        ic = lax.broadcasted_iota(jnp.int32, (128, 128), 1)
        ind = jnp.where((ir >= ic * DH) & (ir < ic * DH + DH) & (ic < GH), 1.0, 0.0).astype(BF16)

        def knorm_max(kf):
            n2 = jnp.dot((kf * kf).astype(BF16), ind, preferred_element_type=F32)
            return jnp.max(n2, axis=0, keepdims=True)

        xa = xa_ref[...]
        qt = lax.dot_general(wqkv_ref[:, 0:D], xa, (((0,), (1,)), ((), ())),
                             preferred_element_type=F32)
        qa_ref[0:D, :] = _bf(qt * QSCALE)
        qa_ref[D:, :] = jnp.zeros((NG * 128 - D, S), F32)
        vt = lax.dot_general(wqkv_ref[:, 2 * D:3 * D], xa, (((0,), (1,)), ((), ())),
                             preferred_element_type=F32)
        vt = _bf(vt)
        ones = jnp.where(row24[DH:] == DH, 1.0, 0.0) * jnp.ones((1, S), F32)
        for h in range(H):
            vta_ref[h, 0:DH, :] = vt[h * DH:(h + 1) * DH, :]
            vta_ref[h, DH:RP, :] = ones
        for g in range(NG):
            kg = jnp.dot(xa, wqkv_ref[:, D + g * GW:D + g * GW + 128], preferred_element_type=F32)
            kg = _bf(kg)
            km = knorm_max(kg)
            for j in range(GH):
                if g * GH + j < H:
                    kmax_ref[g * GH + j] = jnp.max(jnp.where(lane == j, km, 0.0))
            ka_ref[g] = jnp.where(lane == 127, 1.0, kg).astype(BF16)
        xb = xb_ref[...]
        qt = lax.dot_general(wqb_ref[...], xb, (((0,), (1,)), ((), ())),
                             preferred_element_type=F32)
        qb_ref[0:D, :] = _bf(qt * QSCALE)
        qb_ref[D:, :] = jnp.zeros((NG * 128 - D, S), F32)
        vt = lax.dot_general(wvb_ref[...], xb, (((0,), (1,)), ((), ())),
                             preferred_element_type=F32)
        vtb_ref[0:DH, :] = _bf(vt)
        vtb_ref[DH:RP, :] = ones
        wk = wkb_ref[...].astype(F32)
        wk6 = jnp.concatenate([wk] * GH + [jnp.zeros((D, 128 - GW), F32)], axis=1).astype(BF16)
        kg = _bf(jnp.dot(xb, wk6, preferred_element_type=F32))
        km = knorm_max(kg)
        kmax_ref[H] = jnp.max(jnp.where(lane == 0, km, 0.0))
        kb_ref[...] = jnp.where(lane == 127, 1.0, kg).astype(BF16)
        for wo_ref, wop_ref in ((woa_ref, wopa_ref), (wob_ref, wopb_ref)):
            wo = wo_ref[...].astype(F32)
            z = jnp.zeros((RP - DH, D), F32)
            parts = []
            for h in range(H):
                parts.append(wo[h * DH:(h + 1) * DH, :])
                parts.append(z)
            wop_ref[...] = jnp.concatenate(parts, axis=0).astype(BF16)
        bound = jnp.float32(0.0)
        for q_ref, off in ((qa_ref, None), (qb_ref, H)):
            for h in range(H):
                q = q_ref[h * DH:(h + 1) * DH, :]
                qn2 = jnp.max(jnp.sum(q * q, axis=0, keepdims=True))
                bound = jnp.maximum(bound, qn2 * kmax_ref[h if off is None else off])
        flag_ref[0] = (bound * 1.02 < SAFE_BOUND * SAFE_BOUND).astype(jnp.int32)

    qoff = pl.multiple_of(step * TQ, TQ)
    rows = lax.broadcasted_iota(jnp.int32, (128, 1), 0)

    def make_w(q_ref, g, j, k2max, with_bound):
        qg = q_ref[pl.ds(pl.multiple_of(g * GW, 8), 128), pl.ds(qoff, TQ)]
        w = jnp.where((rows >= j * DH) & (rows < j * DH + DH), qg, 0.0)
        if with_bound:
            m = jnp.sqrt(jnp.sum(w * w, axis=0, keepdims=True) * (k2max * 1.02))
            w = jnp.where(rows == 127, -m, w)
        return w.astype(BF16)

    def finish(acc, ot_ref, h):
        inv = 1.0 / acc[DH:DH + 1, :]
        ot_ref[h] = acc * inv

    def fast_head(h, carry):
        g = h // GH
        j = h - g * GH
        wa = make_w(qa_ref, g, j, kmax_ref[h], True)
        wb = make_w(qb_ref, g, j, kmax_ref[H], True)
        n = S // TK
        tasks = []
        for c in range(n):
            tasks.append((0, c))
            tasks.append((1, c))
        acc = [None, None]
        pend = []

        def qk(t):
            b, c = t
            if b == 0:
                k = ka_ref[g, c * TK:(c + 1) * TK, :]
                s = jnp.dot(k, wa, preferred_element_type=F32)
            else:
                k = kb_ref[c * TK:(c + 1) * TK, :]
                s = jnp.dot(k, wb, preferred_element_type=F32)
            return jnp.exp2(s).astype(BF16)

        def pv(t, p):
            b, c = t
            if b == 0:
                v = vta_ref[h, :, c * TK:(c + 1) * TK]
            else:
                v = vtb_ref[:, c * TK:(c + 1) * TK]
            o = lax.dot_general(v, p, (((1,), (0,)), ((), ())), preferred_element_type=F32)
            acc[b] = o if acc[b] is None else acc[b] + o

        depth = 2
        for i in range(len(tasks) + depth):
            if i < len(tasks):
                pend.append((tasks[i], qk(tasks[i])))
            if i >= depth:
                t, p = pend.pop(0)
                pv(t, p)
        finish(acc[0], ota_ref, h)
        finish(acc[1], otb_ref, h)
        return carry

    def slow_head(h, carry):
        g = h // GH
        j = h - g * GH
        for b in range(2):
            w = make_w(qa_ref if b == 0 else qb_ref, g, j, None, False)
            k = ka_ref[g] if b == 0 else kb_ref[...]
            s = jnp.dot(k, w, preferred_element_type=F32)
            m = jnp.max(s, axis=0, keepdims=True)
            p = jnp.exp2(s - m).astype(BF16)
            v = vta_ref[h] if b == 0 else vtb_ref[...]
            o = lax.dot_general(v, p, (((1,), (0,)), ((), ())), preferred_element_type=F32)
            finish(o, ota_ref if b == 0 else otb_ref, h)
        return carry

    @pl.when(flag_ref[0] == 1)
    def _():
        lax.fori_loop(0, H, fast_head, 0)

    @pl.when(flag_ref[0] != 1)
    def _():
        lax.fori_loop(0, H, slow_head, 0)

    for b, (ot_ref, wop_ref) in enumerate(((ota_ref, wopa_ref), (otb_ref, wopb_ref))):
        ot = ot_ref[...].reshape(H * RP, TQ).astype(BF16)
        out = lax.dot_general(ot, wop_ref[...], (((0,), (0,)), ((), ())), preferred_element_type=F32)
        o_ref[:, b * D:(b + 1) * D] = out.astype(o_ref.dtype)


@jax.jit
def pallas_concat_heads__softmax_full_mha__grouped_kv_mqa__prompt_kernel(A_x, A_wqkv, A_wo, B_x, B_wq, B_wk, B_wv, B_wo):
    xa = A_x.reshape(S, D)
    xb = B_x.reshape(S, D)
    full = lambda shape: pl.BlockSpec(shape, lambda i: (0,) * len(shape))
    out = pl.pallas_call(
        _kernel,
        grid=(S // TQ,),
        in_specs=[full((S, D)), full((D, 3 * D)), full((D, D)),
                  full((S, D)), full((D, D)), full((D, DH)), full((D, DH)), full((D, D))],
        out_specs=pl.BlockSpec((TQ, 2 * D), lambda i: (i, 0)),
        out_shape=jax.ShapeDtypeStruct((S, 2 * D), BF16),
        scratch_shapes=[
            pltpu.VMEM((NG * 128, S), F32),
            pltpu.VMEM((NG, S, 128), BF16),
            pltpu.VMEM((H, RP, S), F32),
            pltpu.VMEM((NG * 128, S), F32),
            pltpu.VMEM((S, 128), BF16),
            pltpu.VMEM((RP, S), F32),
            pltpu.VMEM((H, RP, TQ), F32),
            pltpu.VMEM((H, RP, TQ), F32),
            pltpu.VMEM((H * RP, D), BF16),
            pltpu.VMEM((H * RP, D), BF16),
            pltpu.SMEM((H + 1,), F32),
            pltpu.SMEM((1,), jnp.int32),
        ],
        compiler_params=pltpu.CompilerParams(
            dimension_semantics=("arbitrary",),
            vmem_limit_bytes=110 * 1024 * 1024),
    )(xa, A_wqkv, A_wo, xb, B_wq, B_wk, B_wv, B_wo)
    return out.reshape(1, S, 2 * D)
```

```python
import math

import jax
import jax.numpy as jnp
from jax import lax
import jax.experimental.pallas as pl
import jax.experimental.pallas.tpu as pltpu

S = 2048
D = 640
H = 32
DH = 20
RP = 24
TQ = 2048
QW = 512
TK = 128
TS = 512
NT_ = S // TS
KV = NT_ * TK
KB = 64
QB = 128
DEPTH = 2
SLAB = 16
NRING = 8
TO = 256
NFIRST = 2
HEAD_T = 200
TAIL_T = 50
PVW = 24
QSCALE = (DH ** -0.5) * math.log2(math.e)
SAFE_BOUND = 48.0
F32 = jnp.float32
BF16 = jnp.bfloat16
U32 = jnp.uint32
NN = (((1,), (0,)), ((), ()))
TN_T = (((0,), (1,)), ((), ()))
NT = (((1,), (1,)), ((), ()))
TN = (((0,), (0,)), ((), ()))


def _bf(x):
    return x.astype(BF16).astype(F32)


def _dot(a, b, dims=NN):
    return lax.dot_general(a, b, dims, preferred_element_type=F32)


def _kernel(xa_hbm, wqkv_hbm, woa_hbm, xb_hbm, wqb_hbm, wkb_ref, wvb_ref, wob_hbm,
            out_hbm,
            x_ref, w_ref, qp_ref, k_u, vt_ref, kbc_ref, qbc_ref, pv_u, p_u, pd_u, o_ref,
            kt_u, ob_ref, sems, osems):
    nstep = S // TQ
    k_ref = k_u.bitcast(BF16)
    pv_ref = pv_u.bitcast(BF16)
    p_ref = p_u.bitcast(BF16)
    pd_ref = pd_u.bitcast(BF16)
    kt_ref = kt_u.bitcast(BF16)

    def x_copy(b, t):
        src = xa_hbm if b == 0 else xb_hbm
        return pltpu.make_async_copy(src.at[pl.ds(t * TS, TS), :],
                                     x_ref.at[b, pl.ds(t * TS, TS), :], sems.at[b * NT_ + t])

    w_srcs = [wqkv_hbm.at[:, D:2 * D], wqkv_hbm.at[:, 0:D], wqkv_hbm.at[:, 2 * D:3 * D],
              wqb_hbm, woa_hbm, wob_hbm]

    def w_copy(i):
        return pltpu.make_async_copy(w_srcs[i], w_ref.at[i], sems.at[2 * NT_ + i])

    w_copy(0).start()
    for t in range(NT_):
        x_copy(0, t).start()
        x_copy(1, t).start()
    for i in range(1, 6):
        w_copy(i).start()

    ir = lax.broadcasted_iota(jnp.int32, (H, D), 0)
    ic = lax.broadcasted_iota(jnp.int32, (H, D), 1)
    ind = jnp.where((ic >= ir * DH) & (ic < ir * DH + DH), 1.0, 0.0).astype(BF16)

    w_copy(0).wait()

    def proj_k(t, carry):
        kma, kmb = carry
        tile = pl.ds(pl.multiple_of(t * TS, TS), TS)
        half = pl.ds(pl.multiple_of(t * (TS // 2), TS // 2), TS // 2)
        x_copy(0, t).wait()
        x_copy(1, t).wait()
        c4 = lax.broadcasted_iota(jnp.int32, (TS // 2, RP - DH), 1)
        kpad_u = jnp.where(c4 == 0, jnp.uint32(0x3F803F80), jnp.uint32(0))
        kb16 = _dot(x_ref[0, tile, :], w_ref[0]).astype(BF16)
        kt_ref[...] = kb16
        k = kb16.astype(F32)
        kma = jnp.maximum(kma, _dot(ind, (k * k).astype(BF16), NT))
        ku = kt_u[...]
        for h in range(H):
            k_u[half, h * 128:h * 128 + RP] = jnp.concatenate(
                [ku[:, h * DH:(h + 1) * DH], kpad_u], axis=1)
        k = _bf(_dot(x_ref[1, tile, :], wkb_ref[...], NT))
        kmb = jnp.maximum(kmb, _dot(jnp.ones((8, DH), BF16), (k * k).astype(BF16), NT))
        c4 = lax.broadcasted_iota(jnp.int32, (TS, RP - DH), 1)
        k = jnp.concatenate([k, jnp.where(c4 == 0, 1.0, 0.0).astype(F32)], axis=1).astype(BF16)
        k_ref[tile, H * 128:H * 128 + RP] = k
        er = lax.broadcasted_iota(jnp.int32, (RP, DH * 128), 0)
        ec = lax.broadcasted_iota(jnp.int32, (RP, DH * 128), 1)
        e = jnp.where((ec >= er * 128) & (ec < er * 128 + 128), 1.0, 0.0).astype(BF16)
        kbc = _dot(k[0:TK], e)
        rows = pl.ds(pl.multiple_of(t * TK, TK), TK)
        for d in range(DH):
            kbc_ref[d, rows, :] = kbc[:, d * 128:(d + 1) * 128]
        return kma, kmb

    kma, kmb = lax.fori_loop(0, NT_, proj_k,
                             (jnp.zeros((H, TS), F32), jnp.zeros((8, TS), F32)))
    kma = jnp.max(kma, axis=1, keepdims=True) * 1.02
    kmb = jnp.max(kmb[0:1], axis=1, keepdims=True) * 1.02

    for i in (1, 2, 3):
        w_copy(i).wait()

    def proj_qv(t, bound):
        tile = pl.ds(pl.multiple_of(t * TS, TS), TS)
        r4 = lax.broadcasted_iota(jnp.int32, (RP - DH, TS), 0)
        vpad = jnp.where(r4 == 0, 1.0, 0.0).astype(F32)
        zpad = jnp.zeros((RP - DH - 1, TS), F32)
        for b, km in ((0, kma), (1, kmb)):
            x = x_ref[b, tile, :]
            qt = _bf(_dot(w_ref[1 if b == 0 else 3], x, TN_T) * QSCALE)
            m = _bf(jnp.sqrt(_dot(ind, (qt * qt).astype(BF16)) * km))
            bound = jnp.maximum(bound, m)
            for h in range(H):
                qp_ref[b, h, :, tile] = jnp.concatenate(
                    [qt[h * DH:(h + 1) * DH], -m[h:h + 1], zpad], axis=0)
            if b == 0:
                vt = _bf(_dot(w_ref[2], x, TN_T))
                for h in range(H):
                    vt_ref[h, :, tile] = jnp.concatenate([vt[h * DH:(h + 1) * DH], vpad], axis=0)
            else:
                vt = _bf(_dot(wvb_ref[...], x, NT))
                vt_ref[H, :, tile] = jnp.concatenate([vt, vpad], axis=0)
        return bound

    bound = lax.fori_loop(0, NT_, proj_qv, jnp.zeros((H, TS), F32))
    safe = jnp.max(bound) < SAFE_BOUND

    def fill_qbc(it):
        hh = it % H
        qo = pl.multiple_of((it // H) * TQ, TQ)
        qf = qp_ref[1, hh, :, pl.ds(qo, TQ)]
        for d in range(DH + 1):
            qbc_ref[d] = jnp.broadcast_to(qf[d:d + 1, :], (8, TQ))

    vchunks = [t * TS for t in range(NT_)]
    mx = []
    for q0 in range(0, TQ, QW):
        a = [(0, c0, q0) for c0 in range(0, S, TK)]
        b = [(1, c0, q0) for c0 in range(0, S, TK) if c0 not in vchunks]
        while a or b:
            if a:
                mx.append(a.pop(0))
            if b:
                mx.append(b.pop(0))
    nm = len(mx)

    def deferred(dd, hv, ho):
        bb, c0, q0 = mx[nm - DEPTH + dd]
        v = vt_ref[hv if bb == 0 else H, :, c0:c0 + TK]
        o_ref[bb, ho, :, q0:q0 + QW] += _dot(v, pd_ref[dd * TK:(dd + 1) * TK, :])

    def make_fast_head(step):
      qoff = step * TQ

      def fast_head(h, carry):
        it = step * H + h
        hv = jnp.maximum(h - 1, 0)
        ho = jnp.where(h == 0, H, h - 1)
        base = pl.multiple_of((h % 2) * NRING * TK, TK)
        pview = p_ref.at[pl.ds(base, NRING * TK), :]
        koff = pl.multiple_of(h * 128, 128)
        st = dict(done=0, t=0.0, tok=None)

        def vpu_gen():
            for g0 in range(0, TQ, QW):
                for r0 in range(0, KV, KB):
                    for q0 in range(g0, g0 + QW, QB):
                        a_ = jnp.broadcast_to(qbc_ref[DH, :, q0:q0 + QB][None], (KB // 8, 8, QB))
                        for d in range(DH):
                            kk = kbc_ref[d, r0:r0 + KB, :].reshape(KB // 8, 8, 128)
                            if QB > 128:
                                kk = jnp.concatenate([kk] * (QB // 128), axis=2)
                            qd = qbc_ref[d, :, q0:q0 + QB]
                            if st['tok'] is not None:
                                tok = st['tok']
                                if QB > 128:
                                    tok = jnp.concatenate([tok] * (QB // 128), axis=1)
                                qd = qd + tok
                                st['tok'] = None
                            a_ = a_ + kk * qd[None]
                            if d == DH - 1:
                                pv_ref[r0:r0 + KB, q0:q0 + QB] = (
                                    jnp.exp2(a_).reshape(KB, QB).astype(BF16))
                            yield

        nsteps = (TQ // QB) * (KV // KB) * DH
        nold = (TQ // QW) * (KV // TK)
        tot = nm * TK + (nm + nold - NFIRST) * PVW + HEAD_T + TAIL_T
        gen = vpu_gen()

        def adv(p):
            want = min(nsteps, int(math.ceil(st['t'] * nsteps / tot)))
            if st['done'] < want and p is not None:
                st['tok'] = jnp.minimum(p[0:8, 0:128], 0.0)
            while st['done'] < want:
                next(gen)
                st['done'] += 1

        acc = {}

        def qk(ii, extra_t):
            bb, c0, q0 = mx[ii]
            w = qp_ref[bb, h, :, qoff + q0:qoff + q0 + QW]
            if bb == 0:
                kk = k_ref[c0:c0 + TK, pl.ds(koff, RP)]
            else:
                kk = k_ref[c0:c0 + TK, H * 128:H * 128 + RP]
            s = _dot(kk, w)
            for r in range(0, TK, SLAB):
                p = jnp.exp2(s[r:r + SLAB])
                if ii >= nm - DEPTH:
                    r0 = (ii - (nm - DEPTH)) * TK + r
                    pd_ref[r0:r0 + SLAB, :] = p.astype(BF16)
                else:
                    r0 = (ii % NRING) * TK + r
                    pview[r0:r0 + SLAB, :] = p.astype(BF16)
                st['t'] += SLAB + extra_t * SLAB / TK
                adv(p)

        def pv(key, bb, c0, src):
            v = vt_ref[h if bb == 0 else H, :, c0:c0 + TK]
            o = _dot(v, src)
            acc[key] = o if key not in acc else acc[key] + o

        def mk_old(g0, j):
            val = pv_ref[j * TK:(j + 1) * TK, g0:g0 + QW]

            def f():
                pv(('old', g0), 1, vchunks[j], val)
                if j == NT_ - 1:
                    o_ref[1, h, :, g0:g0 + QW] = acc.pop(('old', g0))
            return f

        oldj = [mk_old(g0, j) for g0 in range(0, TQ, QW) for j in range(NT_)]
        for f_ in oldj[:NFIRST]:
            f_()
        extra = oldj[NFIRST:] + [(lambda dd=dd: deferred(dd, hv, ho)) for dd in range(DEPTH)]
        st['t'] = HEAD_T
        adv(None)
        lastuse = {}
        for ii in range(nm - DEPTH):
            lastuse[(mx[ii][0], mx[ii][2])] = ii
        for ii in range(nm):
            npv = (1 if extra else 0) + (1 if ii >= DEPTH else 0)
            qk(ii, npv * PVW)
            if extra:
                extra.pop(0)()
            jj = ii - DEPTH
            if jj >= 0:
                bb, c0, q0 = mx[jj]
                r0 = (jj % NRING) * TK
                pv((bb, q0), bb, c0, pview[r0:r0 + TK, :])
                if lastuse[(bb, q0)] == jj:
                    if bb == 1:
                        o_ref[bb, h, :, q0:q0 + QW] += acc.pop((bb, q0))
                    else:
                        o_ref[bb, h, :, q0:q0 + QW] = acc.pop((bb, q0))
        st['t'] = tot
        adv(None)
        assert not acc and not extra and st['done'] == nsteps
        fill_qbc(jnp.minimum(it + 2, nstep * H - 1))
        return carry
      return fast_head

    def slow_iter(i, carry):
        h = i // (TQ // QW)
        q0 = pl.multiple_of((i % (TQ // QW)) * QW, QW)
        koff = pl.multiple_of(h * 128, 128)
        for bb in range(2):
            w = qp_ref[bb, h, 0:DH, pl.ds(q0, QW)]
            if bb == 0:
                kk = k_ref[:, pl.ds(koff, DH)]
            else:
                kk = k_ref[:, H * 128:H * 128 + DH]
            s = _dot(kk, w)
            m = jnp.max(s, axis=0, keepdims=True)
            p = jnp.exp2(s - m).astype(BF16)
            o_ref[bb, h, :, pl.ds(q0, QW)] = _dot(vt_ref[h if bb == 0 else H], p)
        return carry

    assert nstep == 1

    @pl.when(safe)
    def _():
        pd_u[...] = jnp.zeros(pd_u.shape, U32)
        o_ref[:, H] = jnp.zeros((2, RP, TQ), F32)
        fill_qbc(1)
        for j in range(NT_):
            kb = k_ref[vchunks[j]:vchunks[j] + TK, H * 128:H * 128 + RP]
            pv_ref[j * TK:(j + 1) * TK, :] = jnp.exp2(_dot(kb, qp_ref[1, 0, :, 0:TQ])).astype(BF16)
        lax.fori_loop(0, H, make_fast_head(0), 0)
        for dd in range(DEPTH):
            deferred(dd, H - 1, H - 1)

    @pl.when(jnp.logical_not(safe))
    def _():
        lax.fori_loop(0, H * (TQ // QW), slow_iter, 0)

    w_copy(4).wait()
    w_copy(5).wait()

    def o_copy(t, slot):
        return pltpu.make_async_copy(ob_ref.at[slot], out_hbm.at[pl.ds(t * TO, TO), :],
                                     osems.at[slot])

    def out_proj(t, carry):
        slot = t % 2
        cols = pl.ds(pl.multiple_of(t * TO, TO), TO)

        @pl.when(t >= 2)
        def _():
            o_copy(t - 2, slot).wait()

        for b in range(2):
            o = o_ref[b, 0:H, :, cols]
            o = o * (1.0 / o[:, DH:DH + 1, :])
            ot = jnp.concatenate([o[h, 0:DH] for h in range(H)], axis=0).astype(BF16)
            ob_ref[slot, :, b * D:(b + 1) * D] = _dot(ot, w_ref[4 + b], TN).astype(BF16)
        o_copy(t, slot).start()
        return carry

    nto = S // TO
    lax.fori_loop(0, nto, out_proj, 0)
    o_copy(nto - 2, 0).wait()
    o_copy(nto - 1, 1).wait()


@jax.jit
def pallas_concat_heads__softmax_full_mha__grouped_kv_mqa__prompt_kernel(A_x, A_wqkv, A_wo, B_x, B_wq, B_wk, B_wv, B_wo):
    xa = A_x.reshape(S, D)
    xb = B_x.reshape(S, D)
    hbm = pl.BlockSpec(memory_space=pl.ANY)
    vm = pl.BlockSpec(memory_space=pltpu.VMEM)
    out = pl.pallas_call(
        _kernel,
        in_specs=[hbm, hbm, hbm, hbm, hbm, vm, vm, hbm],
        out_specs=hbm,
        out_shape=jax.ShapeDtypeStruct((S, 2 * D), BF16),
        scratch_shapes=[
            pltpu.VMEM((2, S, D), BF16),
            pltpu.VMEM((6, D, D), BF16),
            pltpu.VMEM((2, H, RP, S), F32),
            pltpu.VMEM((S // 2, (H + 1) * 128), U32),
            pltpu.VMEM((H + 1, RP, S), F32),
            pltpu.VMEM((DH, KV, 128), F32),
            pltpu.VMEM((DH + 1, 8, TQ), F32),
            pltpu.VMEM((KV // 2, TQ), U32),
            pltpu.VMEM((NRING * TK, QW), U32),
            pltpu.VMEM((DEPTH * TK // 2, QW), U32),
            pltpu.VMEM((2, H + 1, RP, TQ), F32),
            pltpu.VMEM((TS // 2, D), U32),
            pltpu.VMEM((2, TO, 2 * D), BF16),
            pltpu.SemaphoreType.DMA((2 * NT_ + 6,)),
            pltpu.SemaphoreType.DMA((2,)),
        ],
        compiler_params=pltpu.CompilerParams(
            vmem_limit_bytes=120 * 1024 * 1024,
            internal_scratch_in_bytes=0x10000),
    )(xa, A_wqkv, A_wo, xb, B_wq, B_wk.T, B_wv.T, B_wo)
    return out.reshape(1, S, 2 * D)
```

```python
import math

import jax
import jax.numpy as jnp
from jax import lax
import jax.experimental.pallas as pl
import jax.experimental.pallas.tpu as pltpu

S = 2048
D = 640
H = 32
DH = 20
RP = 24
QW = 512
TK = 128
TS = 512
NTS = S // TS
KV = NTS * TK
KB = 64
DEPTH = 3
SLAB = 16
NRING = 8
TO = 256
HEAD_T = 150
PVW = 24
QSCALE = (DH ** -0.5) * math.log2(math.e)
SAFE_BOUND = 32.0
SAFE_V = 2.0 ** -30
F32 = jnp.float32
BF16 = jnp.bfloat16
U32 = jnp.uint32
NN = (((1,), (0,)), ((), ()))
NT = (((1,), (1,)), ((), ()))


def _bf(x):
    return x.astype(BF16).astype(F32)


def _dot(a, b, dims=NN):
    return lax.dot_general(a, b, dims, preferred_element_type=F32)


def _kernel(xa_hbm, wqkv_hbm, woa_hbm, xb_hbm, wqb_hbm, wkb_hbm, wvb_hbm, wob_hbm,
            out_hbm,
            x_ref, w_ref, qp_ref, k_u, vt_ref, kbc_ref, qbc_ref, pv_u, p_u, pd_u, o_ref,
            kt_u, ob_ref, oa_u, wt_u, ws_ref, sems, osems):
    k_ref = k_u.bitcast(BF16)
    pv_ref = pv_u.bitcast(BF16)
    p_ref = p_u.bitcast(BF16)
    pd_ref = pd_u.bitcast(BF16)
    kt_ref = kt_u.bitcast(BF16)
    oa_ref = oa_u.bitcast(BF16)
    wt_ref = wt_u.bitcast(BF16)

    def x_copy(b, t):
        src = xa_hbm if b == 0 else xb_hbm
        return pltpu.make_async_copy(src.at[pl.ds(t * TS, TS), :],
                                     x_ref.at[b, pl.ds(t * TS, TS), :], sems.at[b * NTS + t])

    w_srcs = [wqkv_hbm.at[:, D:2 * D], wqkv_hbm.at[:, 0:D], wqkv_hbm.at[:, 2 * D:3 * D],
              wqb_hbm, woa_hbm, wob_hbm]

    def w_copy(i):
        return pltpu.make_async_copy(w_srcs[i], w_ref.at[i], sems.at[2 * NTS + i])

    s_copies = [pltpu.make_async_copy(src, ws_ref.at[i], sems.at[2 * NTS + 6 + i])
                for i, src in enumerate((wkb_hbm, wvb_hbm))]
    for c in s_copies:
        c.start()
    w_copy(0).start()
    for t in range(NTS):
        x_copy(0, t).start()
        x_copy(1, t).start()
    for i in range(1, 6):
        w_copy(i).start()

    ir = lax.broadcasted_iota(jnp.int32, (H, D), 0)
    ic = lax.broadcasted_iota(jnp.int32, (H, D), 1)
    ind = jnp.where((ic >= ir * DH) & (ic < ir * DH + DH), 1.0, 0.0).astype(BF16)

    w_copy(0).wait()
    for c in s_copies:
        c.wait()
    zw = jnp.zeros((RP - DH, D), F32)
    wkv = jnp.concatenate([ws_ref[0].astype(F32), zw, ws_ref[1].astype(F32), zw],
                          axis=0).astype(BF16)

    def proj_k(t, carry):
        kma, kmb, vmb = carry
        tile = pl.ds(pl.multiple_of(t * TS, TS), TS)
        half = pl.ds(pl.multiple_of(t * (TS // 2), TS // 2), TS // 2)
        x_copy(0, t).wait()
        x_copy(1, t).wait()
        r48 = lax.broadcasted_iota(jnp.int32, (2 * RP, TS), 0)
        kv = _bf(_dot(wkv, x_ref[1, tile, :], NT))
        kmb = jnp.maximum(kmb, jnp.sum(kv[0:RP] * kv[0:RP], axis=0, keepdims=True))
        vmb = jnp.maximum(vmb, jnp.abs(kv[RP:2 * RP]))
        kv = jnp.where((r48 == DH) | (r48 == RP + DH), 1.0, kv)
        vt_ref[H, :, tile] = kv[RP:2 * RP]
        kb = jnp.concatenate([kv[0:RP], jnp.zeros((128 - RP, TS), F32)], axis=0).T
        kb = kb[:, 0:RP].astype(BF16)
        k_ref[tile, H * 128:H * 128 + RP] = kb
        c4 = lax.broadcasted_iota(jnp.int32, (TS // 2, RP - DH), 1)
        kpad_u = jnp.where(c4 == 0, jnp.uint32(0x3F803F80), jnp.uint32(0))
        kb16 = _dot(x_ref[0, tile, :], w_ref[0]).astype(BF16)
        kt_ref[...] = kb16
        k = kb16.astype(F32)
        ku = kt_u[...]
        for h in range(H):
            k_u[half, h * 128:h * 128 + RP] = jnp.concatenate(
                [ku[:, h * DH:(h + 1) * DH], kpad_u], axis=1)
        er = lax.broadcasted_iota(jnp.int32, (RP, DH * 128), 0)
        ec = lax.broadcasted_iota(jnp.int32, (RP, DH * 128), 1)
        e = jnp.where((ec >= er * 128) & (ec < er * 128 + 128), 1.0, 0.0).astype(BF16)
        kbc = _dot(kb[0:TK], e)
        rows = pl.ds(pl.multiple_of(t * TK, TK), TK)
        for d in range(DH):
            kbc_ref[d, rows, :] = kbc[:, d * 128:(d + 1) * 128]
        kma = jnp.maximum(kma, _dot(ind, (k * k).astype(BF16), NT))
        return kma, kmb, vmb

    kma, kmb, vmb = lax.fori_loop(
        0, NTS, proj_k,
        (jnp.zeros((H, TS), F32), jnp.zeros((1, TS), F32), jnp.zeros((RP, TS), F32)))
    kma = jnp.max(kma, axis=1, keepdims=True) * 1.02
    kmb = jnp.max(kmb, axis=1, keepdims=True) * 1.02

    for i in (1, 2, 3):
        w_copy(i).wait()
    for i in (1, 2, 3):
        wt_ref[(i - 1) * D:i * D, :] = w_ref[i].T

    def proj_qv(t, carry):
        bound, vma = carry
        tile = pl.ds(pl.multiple_of(t * TS, TS), TS)
        r4 = lax.broadcasted_iota(jnp.int32, (RP - DH, TS), 0)
        vpad = jnp.where(r4 == 0, 1.0, 0.0).astype(F32)
        zpad = jnp.zeros((RP - DH - 1, TS), F32)

        def q_mm(b):
            r0 = 0 if b == 0 else 2 * D
            return _bf(_dot(wt_ref[r0:r0 + D, :], x_ref[b, tile, :], NT) * QSCALE)

        def q_fin(b, qt, km, bound):
            m = _bf(jnp.sqrt(_dot(ind, (qt * qt).astype(BF16)) * km))
            for h in range(H):
                qp_ref[b, h, :, tile] = jnp.concatenate(
                    [qt[h * DH:(h + 1) * DH], -m[h:h + 1], zpad], axis=0)
            return jnp.maximum(bound, m)

        def v_part(c0, c1):
            return _bf(_dot(wt_ref[D + c0:D + c1, :], x_ref[0, tile, :], NT))

        qb = q_mm(1)
        qa = q_mm(0)
        bound = q_fin(1, qb, kmb, bound)
        v0 = v_part(0, 256)
        bound = q_fin(0, qa, kma, bound)
        v1 = v_part(256, D)
        vt = jnp.concatenate([v0, v1], axis=0)
        vma = jnp.maximum(vma, jnp.max(jnp.abs(vt).reshape(D // 8, 8, TS), axis=0))
        for h in range(H):
            vt_ref[h, :, tile] = jnp.concatenate([vt[h * DH:(h + 1) * DH], vpad], axis=0)
        qf = qp_ref[1, 0, :, tile]
        for d in range(DH + 1):
            qbc_ref[d, :, tile] = jnp.broadcast_to(qf[d:d + 1, :], (8, TS))
        pv_u[:, tile] = jnp.zeros((KV // 2, TS), U32)
        o_ref[:, H, :, tile] = jnp.zeros((2, RP, TS), F32)
        return bound, vma

    bound, vma = lax.fori_loop(0, NTS, proj_qv,
                               (jnp.zeros((H, TS), F32), jnp.zeros((8, TS), F32)))
    safe = jnp.logical_and(
        jnp.max(bound) < SAFE_BOUND,
        jnp.minimum(jnp.max(vma), jnp.max(vmb)) > SAFE_V)

    vchunks = [t * TS for t in range(NTS)]
    mx = []
    for q0 in range(0, S, QW):
        a = [(0, c0, q0) for c0 in range(0, S, TK)]
        b = [(1, c0, q0) for c0 in range(0, S, TK) if c0 not in vchunks]
        while a or b:
            if a:
                mx.append(a.pop(0))
            if b:
                mx.append(b.pop(0))
    nm = len(mx)

    def deferred(dd, hv, ho):
        bb, c0, q0 = mx[nm - DEPTH + dd]
        v = vt_ref[hv if bb == 0 else H, :, c0:c0 + TK]
        o_ref[bb, ho, :, q0:q0 + QW] += _dot(v, pd_ref[dd * TK:(dd + 1) * TK, :])

    def fast_head(h, carry):
        hv = jnp.maximum(h - 1, 0)
        ho = jnp.where(h == 0, H, h - 1)
        base = pl.multiple_of((h % 2) * NRING * TK, TK)
        pview = p_ref.at[pl.ds(base, NRING * TK), :]
        koff = pl.multiple_of(h * 128, 128)
        st = dict(done=0, t=float(HEAD_T), tok=None)

        def vpu_gen():
            for g0 in range(0, S, QW):
                for r0 in range(0, KV, KB):
                    for q0 in range(g0, g0 + QW, 128):
                        a_ = jnp.broadcast_to(qbc_ref[DH, :, q0:q0 + 128][None], (KB // 8, 8, 128))
                        for d in range(DH):
                            kk = kbc_ref[d, r0:r0 + KB, :].reshape(KB // 8, 8, 128)
                            qd = qbc_ref[d, :, q0:q0 + 128]
                            if st['tok'] is not None:
                                qd = qd + st['tok']
                                st['tok'] = None
                            a_ = a_ + kk * qd[None]
                            if d == DH - 1:
                                pv_ref[r0:r0 + KB, q0:q0 + 128] = (
                                    jnp.exp2(a_).reshape(KB, 128).astype(BF16))
                            yield

        nsteps = (S // 128) * (KV // KB) * DH
        nold = (S // QW) * NTS
        tot = nm * TK + (nm + nold) * PVW + HEAD_T
        gen = vpu_gen()

        def adv(p):
            want = min(nsteps, int(math.ceil(st['t'] * nsteps / tot)))
            if st['done'] < want and p is not None:
                st['tok'] = jnp.minimum(p[0:8, 0:128], 0.0)
            while st['done'] < want:
                next(gen)
                st['done'] += 1

        acc = {}

        def qk(ii, extra_t):
            bb, c0, q0 = mx[ii]
            w = qp_ref[bb, h, :, q0:q0 + QW]
            if bb == 0:
                kk = k_ref[c0:c0 + TK, pl.ds(koff, RP)]
            else:
                kk = k_ref[c0:c0 + TK, H * 128:H * 128 + RP]
            s = _dot(kk, w)
            for r in range(0, TK, SLAB):
                p = jnp.exp2(s[r:r + SLAB])
                if ii >= nm - DEPTH:
                    r0 = (ii - (nm - DEPTH)) * TK + r
                    pd_ref[r0:r0 + SLAB, :] = p.astype(BF16)
                else:
                    r0 = (ii % NRING) * TK + r
                    pview[r0:r0 + SLAB, :] = p.astype(BF16)
                st['t'] += SLAB + extra_t * SLAB / TK
                adv(p)

        def pv(key, bb, c0, src):
            v = vt_ref[h if bb == 0 else H, :, c0:c0 + TK]
            o = _dot(v, src)
            acc[key] = o if key not in acc else acc[key] + o

        def mk_old(g0, j):
            val = pv_ref[j * TK:(j + 1) * TK, g0:g0 + QW]

            def f():
                pv(('old', g0), 1, vchunks[j], val)
                if j == NTS - 1:
                    o_ref[1, ho, :, g0:g0 + QW] += acc.pop(('old', g0))
            return f

        extra = [mk_old(g0, j) for g0 in range(0, S, QW) for j in range(NTS)]
        extra += [(lambda dd=dd: deferred(dd, hv, ho)) for dd in range(DEPTH)]
        adv(None)
        lastuse = {}
        for ii in range(nm - DEPTH):
            lastuse[(mx[ii][0], mx[ii][2])] = ii
        for ii in range(nm):
            nex = min(len(extra), 2 if ii < DEPTH else 1)
            npv = nex + (1 if ii >= DEPTH else 0)
            qk(ii, npv * PVW)
            for _ in range(nex):
                extra.pop(0)()
            jj = ii - DEPTH
            if jj >= 0:
                bb, c0, q0 = mx[jj]
                r0 = (jj % NRING) * TK
                pv((bb, q0), bb, c0, pview[r0:r0 + TK, :])
                if lastuse[(bb, q0)] == jj:
                    o_ref[bb, h, :, q0:q0 + QW] = acc.pop((bb, q0))
        st['t'] = tot
        adv(None)
        assert not acc and not extra and st['done'] == nsteps
        qf = qp_ref[1, jnp.minimum(h + 1, H - 1)]
        for d in range(DH + 1):
            qbc_ref[d] = jnp.broadcast_to(qf[d:d + 1, :], (8, S))
        return carry

    def slow_iter(i, carry):
        h = i // (S // QW)
        q0 = pl.multiple_of((i % (S // QW)) * QW, QW)
        koff = pl.multiple_of(h * 128, 128)
        for bb in range(2):
            w = qp_ref[bb, h, 0:DH, pl.ds(q0, QW)]
            if bb == 0:
                kk = k_ref[:, pl.ds(koff, DH)]
            else:
                kk = k_ref[:, H * 128:H * 128 + DH]
            s = _dot(kk, w)
            m = jnp.max(s, axis=0, keepdims=True)
            p = jnp.exp2(s - m).astype(BF16)
            o_ref[bb, h, :, pl.ds(q0, QW)] = _dot(vt_ref[h if bb == 0 else H], p)
        return carry

    @pl.when(safe)
    def _():
        pd_u[...] = jnp.zeros(pd_u.shape, U32)
        lax.fori_loop(0, H, fast_head, 0)
        for dd in range(DEPTH):
            deferred(dd, H - 1, H - 1)
        vb = jnp.concatenate([vt_ref[H, :, c0:c0 + TK] for c0 in vchunks], axis=1)
        o_ref[1, H - 1] += _dot(vb, pv_ref[...])

    @pl.when(jnp.logical_not(safe))
    def _():
        lax.fori_loop(0, H * (S // QW), slow_iter, 0)

    w_copy(4).wait()
    w_copy(5).wait()
    nto = S // TO

    def o_copy(t, slot):
        return pltpu.make_async_copy(ob_ref.at[slot], out_hbm.at[pl.ds(t * TO, TO), :],
                                     osems.at[slot])

    def prep(b, t):
        cols = pl.ds(pl.multiple_of(t * TO, TO), TO)
        o = o_ref[b, 0:H, :, cols]
        o = o * (1.0 / o[:, DH:DH + 1, :])
        ot = jnp.concatenate([o[h, 0:DH] for h in range(H)], axis=0).astype(BF16)
        return ot.T

    oa_ref[...] = prep(0, 0)

    def out_proj(t, carry):
        slot = t % 2

        @pl.when(t >= 2)
        def _():
            o_copy(t - 2, slot).wait()

        ob_ref[slot, :, 0:D] = _dot(oa_ref[...], w_ref[4]).astype(BF16)
        ob_ref[slot, :, D:2 * D] = _dot(prep(1, t), w_ref[5]).astype(BF16)
        oa_ref[...] = prep(0, jnp.minimum(t + 1, nto - 1))
        o_copy(t, slot).start()
        return carry

    lax.fori_loop(0, nto, out_proj, 0)
    o_copy(nto - 2, 0).wait()
    o_copy(nto - 1, 1).wait()


@jax.jit
def pallas_concat_heads__softmax_full_mha__grouped_kv_mqa__prompt_kernel(A_x, A_wqkv, A_wo, B_x, B_wq, B_wk, B_wv, B_wo):
    hbm = pl.BlockSpec(memory_space=pl.ANY)
    out = pl.pallas_call(
        _kernel,
        in_specs=[hbm] * 8,
        out_specs=hbm,
        out_shape=jax.ShapeDtypeStruct((S, 2 * D), BF16),
        scratch_shapes=[
            pltpu.VMEM((2, S, D), BF16),
            pltpu.VMEM((6, D, D), BF16),
            pltpu.VMEM((2, H, RP, S), F32),
            pltpu.VMEM((S // 2, (H + 1) * 128), U32),
            pltpu.VMEM((H + 1, RP, S), F32),
            pltpu.VMEM((DH, KV, 128), F32),
            pltpu.VMEM((DH + 1, 8, S), F32),
            pltpu.VMEM((KV // 2, S), U32),
            pltpu.VMEM((NRING * TK, QW), U32),
            pltpu.VMEM((DEPTH * TK // 2, QW), U32),
            pltpu.VMEM((2, H + 1, RP, S), F32),
            pltpu.VMEM((TS // 2, D), U32),
            pltpu.VMEM((2, TO, 2 * D), BF16),
            pltpu.VMEM((TO // 2, D), U32),
            pltpu.VMEM((3 * D // 2, D), U32),
            pltpu.VMEM((2, DH, D), BF16),
            pltpu.SemaphoreType.DMA((2 * NTS + 8,)),
            pltpu.SemaphoreType.DMA((2,)),
        ],
        compiler_params=pltpu.CompilerParams(
            vmem_limit_bytes=120 * 1024 * 1024,
            internal_scratch_in_bytes=0x10000),
    )(A_x.reshape(S, D), A_wqkv, A_wo, B_x.reshape(S, D), B_wq, B_wk.T, B_wv.T, B_wo)
    return out.reshape(1, S, 2 * D)
```

```python
import math

import jax
import jax.numpy as jnp
from jax import lax
import jax.experimental.pallas as pl
import jax.experimental.pallas.tpu as pltpu

S = 2048
D = 640
H = 32
DH = 20
RP = 24
QW = 512
TK = 128
TS = 512
NTS = S // TS
KV = NTS * TK
KB = 64
DEPTH = 3
SLAB = 16
NRING = 8
TO = 256
HEAD_T = 200
PVW = 28
OLD_LEAD = 4
RB = 256
HB = 4
QSCALE = (DH ** -0.5) * math.log2(math.e)
SAFE_BOUND = 32.0
SAFE_V = 2.0 ** -30
F32 = jnp.float32
BF16 = jnp.bfloat16
U32 = jnp.uint32
NN = (((1,), (0,)), ((), ()))
NT = (((1,), (1,)), ((), ()))


def _bf(x):
    return x.astype(BF16).astype(F32)


def _dot(a, b, dims=NN):
    return lax.dot_general(a, b, dims, preferred_element_type=F32)


def _kernel(xa_hbm, wqkv_hbm, woa_hbm, xb_hbm, wqb_hbm, wkb_hbm, wvb_hbm, wob_hbm,
            out_hbm,
            x_ref, w_ref, qp_ref, k_u, vt_ref, kbc_ref, qbc_ref, pv_u, p_u, pd_u, o_ref,
            kt_u, ob_ref, oa_u, wt_u, ws_ref, sems, osems):
    k_ref = k_u.bitcast(BF16)
    pv_ref = pv_u.bitcast(BF16)
    p_ref = p_u.bitcast(BF16)
    pd_ref = pd_u.bitcast(BF16)
    kt_ref = kt_u.bitcast(BF16)
    oa_ref = oa_u.bitcast(BF16)
    wt_ref = wt_u.bitcast(BF16)

    def x_copy(b, t):
        src = xa_hbm if b == 0 else xb_hbm
        return pltpu.make_async_copy(src.at[pl.ds(t * TS, TS), :],
                                     x_ref.at[b, pl.ds(t * TS, TS), :], sems.at[b * NTS + t])

    w_srcs = [wqkv_hbm.at[:, D:2 * D], wqkv_hbm.at[:, 0:D], wqkv_hbm.at[:, 2 * D:3 * D],
              wqb_hbm, woa_hbm, wob_hbm]

    def w_copy(i):
        return pltpu.make_async_copy(w_srcs[i], w_ref.at[i], sems.at[2 * NTS + i])

    s_copies = [pltpu.make_async_copy(src, ws_ref.at[i], sems.at[2 * NTS + 6 + i])
                for i, src in enumerate((wkb_hbm, wvb_hbm))]
    for c in s_copies:
        c.start()
    for t in range(NTS):
        w_copy(t).start()
        x_copy(0, t).start()
        x_copy(1, t).start()
    for i in range(NTS, 6):
        w_copy(i).start()

    pv_u[...] = jnp.zeros(pv_u.shape, U32)
    pd_u[...] = jnp.zeros(pd_u.shape, U32)
    o_ref[:, H] = jnp.zeros((2, RP, S), F32)

    ir = lax.broadcasted_iota(jnp.int32, (H, D), 0)
    ic = lax.broadcasted_iota(jnp.int32, (H, D), 1)
    ind = jnp.where((ic >= ir * DH) & (ic < ir * DH + DH), 1.0, 0.0).astype(BF16)

    for c in s_copies:
        c.wait()
    zw = jnp.zeros((RP - DH, D), F32)
    wkv = jnp.concatenate([ws_ref[0].astype(F32), zw, ws_ref[1].astype(F32), zw],
                          axis=0).astype(BF16)

    def proj_k(t, carry):
        kma, kmb, vmb = carry
        tile = pl.ds(pl.multiple_of(t * TS, TS), TS)
        pltpu.make_async_copy(w_ref.at[t], w_ref.at[t], sems.at[2 * NTS + t]).wait()
        x_copy(0, t).wait()
        x_copy(1, t).wait()
        c4 = lax.broadcasted_iota(jnp.int32, (RB // 2, RP - DH), 1)
        kpad_u = jnp.where(c4 == 0, jnp.uint32(0x3F803F80), jnp.uint32(0))
        ksq = []

        def k_part(r):
            rows = pl.ds(pl.multiple_of(t * TS + r * RB, RB), RB)
            half = pl.ds(pl.multiple_of(t * (TS // 2) + r * (RB // 2), RB // 2), RB // 2)
            kb16 = _dot(x_ref[0, rows, :], w_ref[0]).astype(BF16)
            kt_ref[r * RB:(r + 1) * RB, :] = kb16
            k = kb16.astype(F32)
            ksq.append((k * k).astype(BF16))
            ku = kt_u[r * RB // 2:(r + 1) * RB // 2, :]
            for h in range(H):
                k_u[half, h * 128:h * 128 + RP] = jnp.concatenate(
                    [ku[:, h * DH:(h + 1) * DH], kpad_u], axis=1)

        k_part(0)
        r48 = lax.broadcasted_iota(jnp.int32, (2 * RP, TS), 0)
        kv = _bf(_dot(wkv, x_ref[1, tile, :], NT))
        kmb = jnp.maximum(kmb, jnp.sum(kv[0:RP] * kv[0:RP], axis=0, keepdims=True))
        vmb = jnp.maximum(vmb, jnp.abs(kv[RP:2 * RP]))
        kv = jnp.where((r48 == DH) | (r48 == RP + DH), 1.0, kv)
        vt_ref[H, :, tile] = kv[RP:2 * RP]
        kb = jnp.concatenate([kv[0:RP], jnp.zeros((128 - RP, TS), F32)], axis=0).T
        kb = kb[:, 0:RP].astype(BF16)
        k_ref[tile, H * 128:H * 128 + RP] = kb
        for r in range(1, TS // RB):
            k_part(r)
        wt_ref[pl.ds(pl.multiple_of(t * D, D), D), :] = w_ref[t].T
        er = lax.broadcasted_iota(jnp.int32, (RP, DH * 128), 0)
        ec = lax.broadcasted_iota(jnp.int32, (RP, DH * 128), 1)
        e = jnp.where((ec >= er * 128) & (ec < er * 128 + 128), 1.0, 0.0).astype(BF16)
        kbc = _dot(kb[0:TK], e)
        rows = pl.ds(pl.multiple_of(t * TK, TK), TK)
        for d in range(DH):
            kbc_ref[d, rows, :] = kbc[:, d * 128:(d + 1) * 128]
        kma = jnp.maximum(kma, _dot(ind, jnp.concatenate(ksq, axis=0), NT))
        return kma, kmb, vmb

    kma, kmb, vmb = lax.fori_loop(
        0, NTS, proj_k,
        (jnp.zeros((H, TS), F32), jnp.zeros((1, TS), F32), jnp.zeros((RP, TS), F32)))
    kma = jnp.max(kma, axis=1, keepdims=True) * 1.02
    kmb = jnp.max(kmb, axis=1, keepdims=True) * 1.02
    kma = jnp.broadcast_to(kma, (H, TS))
    kmb = jnp.broadcast_to(kmb, (1, TS))

    def proj_qv(t, carry):
        bound, vma = carry
        tile = pl.ds(pl.multiple_of(t * TS, TS), TS)
        r4 = lax.broadcasted_iota(jnp.int32, (RP - DH, TS), 0)
        vpad = jnp.where(r4 == 0, 1.0, 0.0).astype(F32)
        zpad = jnp.zeros((RP - DH - 1, TS), F32)

        def q_part(b, hb, km, bound):
            r0 = (1 if b == 0 else 3) * D + hb * HB * DH
            qt = _bf(_dot(wt_ref[r0:r0 + HB * DH, :], x_ref[b, tile, :], NT) * QSCALE)
            for j in range(HB):
                h = hb * HB + j
                qh = qt[j * DH:(j + 1) * DH]
                kmh = km[h:h + 1] if b == 0 else km
                m = _bf(jnp.sqrt(jnp.sum(qh * qh, axis=0, keepdims=True) * kmh))
                qp_ref[b, h, :, tile] = jnp.concatenate([qh, -m, zpad], axis=0)
                bound = jnp.maximum(bound, m)
            return bound

        for hb in range(H // HB):
            bound = q_part(1, hb, kmb, bound)
        for hb in range(H // HB):
            bound = q_part(0, hb, kma, bound)
        vt = _bf(_dot(wt_ref[2 * D:3 * D, :], x_ref[0, tile, :], NT))
        vma = jnp.maximum(vma, jnp.max(jnp.abs(vt).reshape(D // 8, 8, TS), axis=0))
        for h in range(H):
            vt_ref[h, :, tile] = jnp.concatenate([vt[h * DH:(h + 1) * DH], vpad], axis=0)
        qf = qp_ref[1, 0, :, tile]
        for d in range(DH + 1):
            qbc_ref[d, :, tile] = jnp.broadcast_to(qf[d:d + 1, :], (8, TS))
        return bound, vma

    bound, vma = lax.fori_loop(0, NTS, proj_qv,
                               (jnp.zeros((1, TS), F32), jnp.zeros((8, TS), F32)))
    safe = jnp.logical_and(
        jnp.max(bound) < SAFE_BOUND,
        jnp.minimum(jnp.max(vma), jnp.max(vmb)) > SAFE_V)

    vchunks = [t * TS for t in range(NTS)]
    mx = []
    for q0 in range(0, S, QW):
        a = [(0, c0, q0) for c0 in range(0, S, TK)]
        b = [(1, c0, q0) for c0 in range(0, S, TK) if c0 not in vchunks]
        while a or b:
            if a:
                mx.append(a.pop(0))
            if b:
                mx.append(b.pop(0))
    nm = len(mx)

    def deferred(dd, hv, ho):
        bb, c0, q0 = mx[nm - DEPTH + dd]
        v = vt_ref[hv if bb == 0 else H, :, c0:c0 + TK]
        o_ref[bb, ho, :, q0:q0 + QW] += _dot(v, pd_ref[dd * TK:(dd + 1) * TK, :])

    def fast_head(h, carry):
        hv = jnp.maximum(h - 1, 0)
        ho = jnp.where(h == 0, H, h - 1)
        base = pl.multiple_of((h % 2) * NRING * TK, TK)
        pview = p_ref.at[pl.ds(base, NRING * TK), :]
        koff = pl.multiple_of(h * 128, 128)
        st = dict(done=0, t=float(HEAD_T), tok=None)

        def vpu_gen():
            for g0 in range(0, S, QW):
                for r0 in range(0, KV, KB):
                    for q0 in range(g0, g0 + QW, 128):
                        a_ = jnp.broadcast_to(qbc_ref[DH, :, q0:q0 + 128][None], (KB // 8, 8, 128))
                        for d in range(DH):
                            kk = kbc_ref[d, r0:r0 + KB, :].reshape(KB // 8, 8, 128)
                            qd = qbc_ref[d, :, q0:q0 + 128]
                            if st['tok'] is not None:
                                qd = qd + st['tok']
                                st['tok'] = None
                            a_ = a_ + kk * qd[None]
                            if d == DH - 1:
                                pv_ref[r0:r0 + KB, q0:q0 + 128] = (
                                    jnp.exp2(a_).reshape(KB, 128).astype(BF16))
                            yield

        nsteps = (S // 128) * (KV // KB) * DH
        nold = (S // QW) * NTS
        tot = nm * TK + (nm + nold) * PVW + HEAD_T
        gen = vpu_gen()

        def adv(p):
            want = min(nsteps, int(math.ceil(st['t'] * nsteps / tot)))
            if st['done'] < want and p is not None:
                st['tok'] = jnp.minimum(p[0:8, 0:128], 0.0)
            while st['done'] < want:
                next(gen)
                st['done'] += 1

        acc = {}

        def qk(ii, extra_t, lo=0, hi=TK):
            bb, c0, q0 = mx[ii]
            w = qp_ref[bb, h, :, q0:q0 + QW]
            if bb == 0:
                kk = k_ref[c0 + lo:c0 + hi, pl.ds(koff, RP)]
            else:
                kk = k_ref[c0 + lo:c0 + hi, H * 128:H * 128 + RP]
            s = _dot(kk, w)
            for r in range(lo, hi, SLAB):
                p = jnp.exp2(s[r - lo:r - lo + SLAB])
                if ii >= nm - DEPTH:
                    r0 = (ii - (nm - DEPTH)) * TK + r
                    pd_ref[r0:r0 + SLAB, :] = p.astype(BF16)
                else:
                    r0 = (ii % NRING) * TK + r
                    pview[r0:r0 + SLAB, :] = p.astype(BF16)
                st['t'] += SLAB + extra_t * SLAB / TK
                adv(p)

        def pv(key, bb, c0, src):
            v = vt_ref[h if bb == 0 else H, :, c0:c0 + TK]
            o = _dot(v, src)
            acc[key] = o if key not in acc else acc[key] + o

        def old_load(n):
            assert st['done'] < n * (nsteps // nold) + DH
            g0, j = (n // NTS) * QW, n % NTS
            return pv_ref[j * TK:(j + 1) * TK, g0:g0 + QW]

        def old_tile(n, val=None):
            g0, j = (n // NTS) * QW, n % NTS
            v = vt_ref[H, :, vchunks[j]:vchunks[j] + TK]
            o_ref[1, ho, :, g0:g0 + QW] += _dot(v, old_load(n) if val is None else val)

        olds = {}
        for n in range(nold):
            olds.setdefault(max(0, (nm * n) // nold - OLD_LEAD), []).append(n)
        val0 = old_load(0)
        adv(None)
        lastuse = {}
        for ii in range(nm - DEPTH):
            lastuse[(mx[ii][0], mx[ii][2])] = ii
        for ii in range(nm):
            ex = olds.pop(ii, [])
            if len(ex) == 1:
                qk(ii, 2 * PVW, 0, TK // 2)
                old_tile(ex[0], val0 if ex[0] == 0 else None)
                qk(ii, 2 * PVW, TK // 2, TK)
            else:
                assert not ex
                qk(ii, PVW)
            jj = ii - DEPTH
            if jj >= 0:
                bb, c0, q0 = mx[jj]
                r0 = (jj % NRING) * TK
                pv((bb, q0), bb, c0, pview[r0:r0 + TK, :])
                if lastuse[(bb, q0)] == jj:
                    o_ref[bb, h, :, q0:q0 + QW] = acc.pop((bb, q0))
            else:
                deferred(ii, hv, ho)
        st['t'] = tot
        adv(None)
        assert not acc and not olds and st['done'] == nsteps
        qf = qp_ref[1, jnp.minimum(h + 1, H - 1)]
        for d in range(DH + 1):
            qbc_ref[d] = jnp.broadcast_to(qf[d:d + 1, :], (8, S))
        return carry

    def slow_iter(i, carry):
        h = i // (S // QW)
        q0 = pl.multiple_of((i % (S // QW)) * QW, QW)
        koff = pl.multiple_of(h * 128, 128)
        for bb in range(2):
            w = qp_ref[bb, h, 0:DH, pl.ds(q0, QW)]
            if bb == 0:
                kk = k_ref[:, pl.ds(koff, DH)]
            else:
                kk = k_ref[:, H * 128:H * 128 + DH]
            s = _dot(kk, w)
            m = jnp.max(s, axis=0, keepdims=True)
            p = jnp.exp2(s - m).astype(BF16)
            o_ref[bb, h, :, pl.ds(q0, QW)] = _dot(vt_ref[h if bb == 0 else H], p)
        return carry

    def prep(b, t):
        cols = pl.ds(t * TO if isinstance(t, int) else pl.multiple_of(t * TO, TO), TO)
        den = jnp.concatenate([o_ref[b, h, DH:DH + 1, cols] for h in range(H)], axis=0)
        inv = 1.0 / den
        ot = jnp.concatenate([o_ref[b, h, 0:DH, cols] * inv[h:h + 1] for h in range(H)], axis=0)
        return ot.astype(BF16).T

    @pl.when(safe)
    def _():
        lax.fori_loop(0, H, fast_head, 0)
        for dd in range(DEPTH):
            deferred(dd, H - 1, H - 1)
        vb = jnp.concatenate([vt_ref[H, :, c0:c0 + TK] for c0 in vchunks], axis=1)
        o_ref[1, H - 1] += _dot(vb, pv_ref[...])
        oa_ref[...] = prep(0, 0)

    @pl.when(jnp.logical_not(safe))
    def _():
        lax.fori_loop(0, H * (S // QW), slow_iter, 0)
        oa_ref[...] = prep(0, 0)

    w_copy(4).wait()
    w_copy(5).wait()
    nto = S // TO

    def o_copy(t, slot):
        return pltpu.make_async_copy(ob_ref.at[slot], out_hbm.at[pl.ds(t * TO, TO), :],
                                     osems.at[slot])

    def out_proj(t, carry):
        slot = t % 2

        @pl.when(t >= 2)
        def _():
            o_copy(t - 2, slot).wait()

        ob_ref[slot, :, 0:D] = _dot(oa_ref[...], w_ref[4]).astype(BF16)
        pb = prep(1, t)
        oa_ref[...] = prep(0, jnp.minimum(t + 1, nto - 1))
        ob_ref[slot, :, D:2 * D] = _dot(pb, w_ref[5]).astype(BF16)
        o_copy(t, slot).start()
        return carry

    lax.fori_loop(0, nto, out_proj, 0)
    o_copy(nto - 2, 0).wait()
    o_copy(nto - 1, 1).wait()


@jax.jit
def pallas_concat_heads__softmax_full_mha__grouped_kv_mqa__prompt_kernel(A_x, A_wqkv, A_wo, B_x, B_wq, B_wk, B_wv, B_wo):
    hbm = pl.BlockSpec(memory_space=pl.ANY)
    out = pl.pallas_call(
        _kernel,
        in_specs=[hbm] * 8,
        out_specs=hbm,
        out_shape=jax.ShapeDtypeStruct((S, 2 * D), BF16),
        scratch_shapes=[
            pltpu.VMEM((2, S, D), BF16),
            pltpu.VMEM((6, D, D), BF16),
            pltpu.VMEM((2, H, RP, S), F32),
            pltpu.VMEM((S // 2, (H + 1) * 128), U32),
            pltpu.VMEM((H + 1, RP, S), F32),
            pltpu.VMEM((DH, KV, 128), F32),
            pltpu.VMEM((DH + 1, 8, S), F32),
            pltpu.VMEM((KV // 2, S), U32),
            pltpu.VMEM((NRING * TK, QW), U32),
            pltpu.VMEM((DEPTH * TK // 2, QW), U32),
            pltpu.VMEM((2, H + 1, RP, S), F32),
            pltpu.VMEM((TS // 2, D), U32),
            pltpu.VMEM((2, TO, 2 * D), BF16),
            pltpu.VMEM((TO // 2, D), U32),
            pltpu.VMEM((4 * D // 2, D), U32),
            pltpu.VMEM((2, DH, D), BF16),
            pltpu.SemaphoreType.DMA((2 * NTS + 8,)),
            pltpu.SemaphoreType.DMA((2,)),
        ],
        compiler_params=pltpu.CompilerParams(
            vmem_limit_bytes=120 * 1024 * 1024,
            internal_scratch_in_bytes=0x40000),
    )(A_x.reshape(S, D), A_wqkv, A_wo, B_x.reshape(S, D), B_wq, B_wk.T, B_wv.T, B_wo)
    return out.reshape(1, S, 2 * D)
```

```python
import math

import jax
import jax.numpy as jnp
from jax import lax
import jax.experimental.pallas as pl
import jax.experimental.pallas.tpu as pltpu

S = 2048
D = 640
H = 32
DH = 20
RP = 24
QW = 512
TK = 128
TS = 512
NTS = S // TS
KV = NTS * TK
KB = 64
DEPTH = 3
SLAB = 16
NRING = 8
TO = 256
HEAD_T = 200
PVW = 28
OLD_LEAD = 4
RB = 256
HB = 4
QSCALE = (DH ** -0.5) * math.log2(math.e)
SAFE_BOUND = 32.0
SAFE_V = 2.0 ** -30
F32 = jnp.float32
BF16 = jnp.bfloat16
U32 = jnp.uint32
NN = (((1,), (0,)), ((), ()))
NT = (((1,), (1,)), ((), ()))


def _bf(x):
    return x.astype(BF16).astype(F32)


def _dot(a, b, dims=NN):
    return lax.dot_general(a, b, dims, preferred_element_type=F32)


def _kernel(xa_hbm, wqkv_hbm, woa_hbm, xb_hbm, wqb_hbm, wkb_hbm, wvb_hbm, wob_hbm,
            out_hbm,
            x_ref, w_ref, qp_ref, k_u, vt_ref, kbc_ref, qbc_ref, pv_u, p_u, pd_u, o_ref,
            kt_u, ob_ref, oa_u, wt_u, ws_ref, sems, osems):
    k_ref = k_u.bitcast(BF16)
    pv_ref = pv_u.bitcast(BF16)
    p_ref = p_u.bitcast(BF16)
    pd_ref = pd_u.bitcast(BF16)
    kt_ref = kt_u.bitcast(BF16)
    oa_ref = oa_u.bitcast(BF16)
    wt_ref = wt_u.bitcast(BF16)

    def x_copy(b, t):
        src = xa_hbm if b == 0 else xb_hbm
        return pltpu.make_async_copy(src.at[pl.ds(t * TS, TS), :],
                                     x_ref.at[b, pl.ds(t * TS, TS), :], sems.at[b * NTS + t])

    w_srcs = [wqkv_hbm.at[:, D:2 * D], wqkv_hbm.at[:, 0:D], wqkv_hbm.at[:, 2 * D:3 * D],
              wqb_hbm, woa_hbm, wob_hbm]

    def w_copy(i):
        return pltpu.make_async_copy(w_srcs[i], w_ref.at[i], sems.at[2 * NTS + i])

    s_copies = [pltpu.make_async_copy(src, ws_ref.at[i], sems.at[2 * NTS + 6 + i])
                for i, src in enumerate((wkb_hbm, wvb_hbm))]
    for c in s_copies:
        c.start()
    for t in range(NTS):
        w_copy(t).start()
        x_copy(0, t).start()
        x_copy(1, t).start()
    for i in range(NTS, 6):
        w_copy(i).start()

    pv_u[...] = jnp.zeros(pv_u.shape, U32)
    pd_u[...] = jnp.zeros(pd_u.shape, U32)
    o_ref[:, H] = jnp.zeros((2, RP, S), F32)

    ir = lax.broadcasted_iota(jnp.int32, (H, D), 0)
    ic = lax.broadcasted_iota(jnp.int32, (H, D), 1)
    ind = jnp.where((ic >= ir * DH) & (ic < ir * DH + DH), 1.0, 0.0).astype(BF16)

    for c in s_copies:
        c.wait()
    zw = jnp.zeros((RP - DH, D), F32)
    wkv = jnp.concatenate([ws_ref[0].astype(F32), zw, ws_ref[1].astype(F32), zw],
                          axis=0).astype(BF16)

    def proj_k(t, carry):
        kma, kmb, vmb = carry
        tile = pl.ds(pl.multiple_of(t * TS, TS), TS)
        pltpu.make_async_copy(w_ref.at[t], w_ref.at[t], sems.at[2 * NTS + t]).wait()
        x_copy(0, t).wait()
        x_copy(1, t).wait()
        c4 = lax.broadcasted_iota(jnp.int32, (RB // 2, RP - DH), 1)
        kpad_u = jnp.where(c4 == 0, jnp.uint32(0x3F803F80), jnp.uint32(0))
        ksq = []

        def k_part(r):
            rows = pl.ds(pl.multiple_of(t * TS + r * RB, RB), RB)
            half = pl.ds(pl.multiple_of(t * (TS // 2) + r * (RB // 2), RB // 2), RB // 2)
            kb16 = _dot(x_ref[0, rows, :], w_ref[0]).astype(BF16)
            kt_ref[r * RB:(r + 1) * RB, :] = kb16
            k = kb16.astype(F32)
            ksq.append((k * k).astype(BF16))
            ku = kt_u[r * RB // 2:(r + 1) * RB // 2, :]
            for h in range(H):
                k_u[half, h * 128:h * 128 + RP] = jnp.concatenate(
                    [ku[:, h * DH:(h + 1) * DH], kpad_u], axis=1)

        k_part(0)
        r48 = lax.broadcasted_iota(jnp.int32, (2 * RP, TS), 0)
        kv = _bf(_dot(wkv, x_ref[1, tile, :], NT))
        kmb = jnp.maximum(kmb, jnp.sum(kv[0:RP] * kv[0:RP], axis=0, keepdims=True))
        vmb = jnp.maximum(vmb, jnp.abs(kv[RP:2 * RP]))
        kv = jnp.where((r48 == DH) | (r48 == RP + DH), 1.0, kv)
        vt_ref[H, :, tile] = kv[RP:2 * RP]
        kb = jnp.concatenate([kv[0:RP], jnp.zeros((128 - RP, TS), F32)], axis=0).T
        kb = kb[:, 0:RP].astype(BF16)
        k_ref[tile, H * 128:H * 128 + RP] = kb
        for r in range(1, TS // RB):
            k_part(r)
        wt_ref[pl.ds(pl.multiple_of(t * D, D), D), :] = w_ref[t].T
        er = lax.broadcasted_iota(jnp.int32, (RP, DH * 128), 0)
        ec = lax.broadcasted_iota(jnp.int32, (RP, DH * 128), 1)
        e = jnp.where((ec >= er * 128) & (ec < er * 128 + 128), 1.0, 0.0).astype(BF16)
        kbc = _dot(kb[0:TK], e)
        rows = pl.ds(pl.multiple_of(t * TK, TK), TK)
        for d in range(DH):
            kbc_ref[d, rows, :] = kbc[:, d * 128:(d + 1) * 128]
        kma = jnp.maximum(kma, _dot(ind, jnp.concatenate(ksq, axis=0), NT))
        return kma, kmb, vmb

    kma, kmb, vmb = lax.fori_loop(
        0, NTS, proj_k,
        (jnp.zeros((H, TS), F32), jnp.zeros((1, TS), F32), jnp.zeros((RP, TS), F32)))
    kma = jnp.max(kma, axis=1, keepdims=True) * 1.02
    kmb = jnp.max(kmb, axis=1, keepdims=True) * 1.02
    kma = jnp.broadcast_to(kma, (H, TS))
    kmb = jnp.broadcast_to(kmb, (1, TS))

    def proj_qv(t, carry):
        bound, vma = carry
        tile = pl.ds(pl.multiple_of(t * TS, TS), TS)
        r4 = lax.broadcasted_iota(jnp.int32, (RP - DH, TS), 0)
        vpad = jnp.where(r4 == 0, 1.0, 0.0).astype(F32)
        zpad = jnp.zeros((RP - DH - 1, TS), F32)

        def q_part(b, hb, km, bound):
            r0 = (1 if b == 0 else 3) * D + hb * HB * DH
            qt = _bf(_dot(wt_ref[r0:r0 + HB * DH, :], x_ref[b, tile, :], NT) * QSCALE)
            for j in range(HB):
                h = hb * HB + j
                qh = qt[j * DH:(j + 1) * DH]
                kmh = km[h:h + 1] if b == 0 else km
                m = _bf(jnp.sqrt(jnp.sum(qh * qh, axis=0, keepdims=True) * kmh))
                qp_ref[b, h, :, tile] = jnp.concatenate([qh, -m, zpad], axis=0)
                bound = jnp.maximum(bound, m)
            return bound

        for hb in range(H // HB):
            bound = q_part(1, hb, kmb, bound)
        for hb in range(H // HB):
            bound = q_part(0, hb, kma, bound)
        vt = _bf(_dot(wt_ref[2 * D:3 * D, :], x_ref[0, tile, :], NT))
        vma = jnp.maximum(vma, jnp.max(jnp.abs(vt).reshape(D // 8, 8, TS), axis=0))
        for h in range(H):
            vt_ref[h, :, tile] = jnp.concatenate([vt[h * DH:(h + 1) * DH], vpad], axis=0)
        qf = qp_ref[1, 0, :, tile]
        for d in range(DH + 1):
            qbc_ref[d, :, tile] = jnp.broadcast_to(qf[d:d + 1, :], (8, TS))
        return bound, vma

    bound, vma = lax.fori_loop(0, NTS, proj_qv,
                               (jnp.zeros((1, TS), F32), jnp.zeros((8, TS), F32)))
    safe = jnp.logical_and(
        jnp.max(bound) < SAFE_BOUND,
        jnp.minimum(jnp.max(vma), jnp.max(vmb)) > SAFE_V)

    vchunks = [t * TS for t in range(NTS)]
    mx = []
    for q0 in range(0, S, QW):
        a = [(0, c0, q0) for c0 in range(0, S, TK)]
        b = [(1, c0, q0) for c0 in range(0, S, TK) if c0 not in vchunks]
        mx += b + a
    nm = len(mx)

    def deferred(dd, hv, ho):
        bb, c0, q0 = mx[nm - DEPTH + dd]
        v = vt_ref[hv if bb == 0 else H, :, c0:c0 + TK]
        o_ref[bb, ho, :, q0:q0 + QW] += _dot(v, pd_ref[dd * TK:(dd + 1) * TK, :])

    def fast_head(h, carry):
        hv = jnp.maximum(h - 1, 0)
        ho = jnp.where(h == 0, H, h - 1)
        base = pl.multiple_of((h % 2) * NRING * TK, TK)
        pview = p_ref.at[pl.ds(base, NRING * TK), :]
        koff = pl.multiple_of(h * 128, 128)
        st = dict(done=0, t=float(HEAD_T), tok=None)

        def vpu_gen():
            for g0 in range(0, S, QW):
                for r0 in range(0, KV, KB):
                    for q0 in range(g0, g0 + QW, 128):
                        a_ = jnp.broadcast_to(qbc_ref[DH, :, q0:q0 + 128][None], (KB // 8, 8, 128))
                        for d in range(DH):
                            kk = kbc_ref[d, r0:r0 + KB, :].reshape(KB // 8, 8, 128)
                            qd = qbc_ref[d, :, q0:q0 + 128]
                            if st['tok'] is not None:
                                qd = qd + st['tok']
                                st['tok'] = None
                            a_ = a_ + kk * qd[None]
                            if d == DH - 1:
                                pv_ref[r0:r0 + KB, q0:q0 + 128] = (
                                    jnp.exp2(a_).reshape(KB, 128).astype(BF16))
                            yield

        nsteps = (S // 128) * (KV // KB) * DH
        nold = (S // QW) * NTS
        tot = nm * TK + (nm + nold) * PVW + HEAD_T
        gen = vpu_gen()

        def adv(p):
            want = min(nsteps, int(math.ceil(st['t'] * nsteps / tot)))
            if st['done'] < want and p is not None:
                st['tok'] = jnp.minimum(p[8:16, 384:512], 0.0)
            while st['done'] < want:
                next(gen)
                st['done'] += 1

        acc = {}

        def qk(ii, extra_t, lo=0, hi=TK):
            bb, c0, q0 = mx[ii]
            w = qp_ref[bb, h, :, q0:q0 + QW]
            if bb == 0:
                kk = k_ref[c0 + lo:c0 + hi, pl.ds(koff, RP)]
            else:
                kk = k_ref[c0 + lo:c0 + hi, H * 128:H * 128 + RP]
            s = _dot(kk, w)
            for r in range(lo, hi, SLAB):
                p = jnp.exp2(s[r - lo:r - lo + SLAB])
                if ii >= nm - DEPTH:
                    r0 = (ii - (nm - DEPTH)) * TK + r
                    pd_ref[r0:r0 + SLAB, :] = p.astype(BF16)
                else:
                    r0 = (ii % NRING) * TK + r
                    pview[r0:r0 + SLAB, :] = p.astype(BF16)
                st['t'] += SLAB + extra_t * SLAB / TK
                adv(p)

        def pv(key, bb, c0, src):
            v = vt_ref[h if bb == 0 else H, :, c0:c0 + TK]
            o = _dot(v, src)
            acc[key] = o if key not in acc else acc[key] + o

        def old_load(n):
            assert st['done'] < n * (nsteps // nold) + DH
            g0, j = (n // NTS) * QW, n % NTS
            return pv_ref[j * TK:(j + 1) * TK, g0:g0 + QW]

        def old_tile(n, val=None):
            g0, j = (n // NTS) * QW, n % NTS
            v = vt_ref[H, :, vchunks[j]:vchunks[j] + TK]
            o_ref[1, ho, :, g0:g0 + QW] += _dot(v, old_load(n) if val is None else val)

        olds = {}
        for n in range(nold):
            olds.setdefault(max(0, (nm * n) // nold - OLD_LEAD), []).append(n)
        val0 = old_load(0)
        adv(None)
        lastuse = {}
        for ii in range(nm - DEPTH):
            lastuse[(mx[ii][0], mx[ii][2])] = ii
        for ii in range(nm):
            ex = olds.pop(ii, [])
            if len(ex) == 1:
                qk(ii, 2 * PVW, 0, TK // 2)
                old_tile(ex[0], val0 if ex[0] == 0 else None)
                qk(ii, 2 * PVW, TK // 2, TK)
            else:
                assert not ex
                qk(ii, PVW)
            jj = ii - DEPTH
            if jj >= 0:
                bb, c0, q0 = mx[jj]
                r0 = (jj % NRING) * TK
                pv((bb, q0), bb, c0, pview[r0:r0 + TK, :])
                if lastuse[(bb, q0)] == jj:
                    o_ref[bb, h, :, q0:q0 + QW] = acc.pop((bb, q0))
            else:
                deferred(ii, hv, ho)
        st['t'] = tot
        adv(None)
        assert not acc and not olds and st['done'] == nsteps
        qf = qp_ref[1, jnp.minimum(h + 1, H - 1)]
        for d in range(DH + 1):
            qbc_ref[d] = jnp.broadcast_to(qf[d:d + 1, :], (8, S))
        return carry

    def slow_iter(i, carry):
        h = i // (S // QW)
        q0 = pl.multiple_of((i % (S // QW)) * QW, QW)
        koff = pl.multiple_of(h * 128, 128)
        for bb in range(2):
            w = qp_ref[bb, h, 0:DH, pl.ds(q0, QW)]
            if bb == 0:
                kk = k_ref[:, pl.ds(koff, DH)]
            else:
                kk = k_ref[:, H * 128:H * 128 + DH]
            s = _dot(kk, w)
            m = jnp.max(s, axis=0, keepdims=True)
            p = jnp.exp2(s - m).astype(BF16)
            o_ref[bb, h, :, pl.ds(q0, QW)] = _dot(vt_ref[h if bb == 0 else H], p)
        return carry

    def prep(b, t):
        cols = pl.ds(t * TO if isinstance(t, int) else pl.multiple_of(t * TO, TO), TO)
        den = jnp.concatenate([o_ref[b, h, DH:DH + 1, cols] for h in range(H)], axis=0)
        inv = 1.0 / den
        ot = jnp.concatenate([o_ref[b, h, 0:DH, cols] * inv[h:h + 1] for h in range(H)], axis=0)
        return ot.astype(BF16).T

    @pl.when(safe)
    def _():
        lax.fori_loop(0, H, fast_head, 0)
        for dd in range(DEPTH):
            deferred(dd, H - 1, H - 1)
        vb = jnp.concatenate([vt_ref[H, :, c0:c0 + TK] for c0 in vchunks], axis=1)
        o_ref[1, H - 1] += _dot(vb, pv_ref[...])
        oa_ref[...] = prep(0, 0)

    @pl.when(jnp.logical_not(safe))
    def _():
        lax.fori_loop(0, H * (S // QW), slow_iter, 0)
        oa_ref[...] = prep(0, 0)

    w_copy(4).wait()
    w_copy(5).wait()
    nto = S // TO

    def o_copy(t, slot):
        return pltpu.make_async_copy(ob_ref.at[slot], out_hbm.at[pl.ds(t * TO, TO), :],
                                     osems.at[slot])

    def out_proj(t, carry):
        slot = t % 2

        @pl.when(t >= 2)
        def _():
            o_copy(t - 2, slot).wait()

        ob_ref[slot, :, 0:D] = _dot(oa_ref[...], w_ref[4]).astype(BF16)
        pb = prep(1, t)
        oa_ref[...] = prep(0, jnp.minimum(t + 1, nto - 1))
        ob_ref[slot, :, D:2 * D] = _dot(pb, w_ref[5]).astype(BF16)
        o_copy(t, slot).start()
        return carry

    lax.fori_loop(0, nto, out_proj, 0)
    o_copy(nto - 2, 0).wait()
    o_copy(nto - 1, 1).wait()


@jax.jit
def pallas_concat_heads__softmax_full_mha__grouped_kv_mqa__prompt_kernel(A_x, A_wqkv, A_wo, B_x, B_wq, B_wk, B_wv, B_wo):
    hbm = pl.BlockSpec(memory_space=pl.ANY)
    out = pl.pallas_call(
        _kernel,
        in_specs=[hbm] * 8,
        out_specs=hbm,
        out_shape=jax.ShapeDtypeStruct((S, 2 * D), BF16),
        scratch_shapes=[
            pltpu.VMEM((2, S, D), BF16),
            pltpu.VMEM((6, D, D), BF16),
            pltpu.VMEM((2, H, RP, S), F32),
            pltpu.VMEM((S // 2, (H + 1) * 128), U32),
            pltpu.VMEM((H + 1, RP, S), F32),
            pltpu.VMEM((DH, KV, 128), F32),
            pltpu.VMEM((DH + 1, 8, S), F32),
            pltpu.VMEM((KV // 2, S), U32),
            pltpu.VMEM((NRING * TK, QW), U32),
            pltpu.VMEM((DEPTH * TK // 2, QW), U32),
            pltpu.VMEM((2, H + 1, RP, S), F32),
            pltpu.VMEM((TS // 2, D), U32),
            pltpu.VMEM((2, TO, 2 * D), BF16),
            pltpu.VMEM((TO // 2, D), U32),
            pltpu.VMEM((4 * D // 2, D), U32),
            pltpu.VMEM((2, DH, D), BF16),
            pltpu.SemaphoreType.DMA((2 * NTS + 8,)),
            pltpu.SemaphoreType.DMA((2,)),
        ],
        compiler_params=pltpu.CompilerParams(
            vmem_limit_bytes=120 * 1024 * 1024,
            internal_scratch_in_bytes=0x40000),
    )(A_x.reshape(S, D), A_wqkv, A_wo, B_x.reshape(S, D), B_wq, B_wk.T, B_wv.T, B_wo)
    return out.reshape(1, S, 2 * D)
```
